```python
import jax
import jax.numpy as jnp

def _softmax(x, axis=-1):
    return jax.nn.softmax(x, axis=axis)

def _gelu(x):
    return jax.nn.gelu(x, approximate=True)

def _silu(x):
    return jax.nn.silu(x)

def _sigmoid(x):
    return jax.nn.sigmoid(x)

def _layernorm(x, axis=-1, eps=1e-05):
    m = jnp.mean(x, axis=axis, keepdims=True)
    v = jnp.var(x, axis=axis, keepdims=True)
    return (x - m) / jnp.sqrt(v + eps)

def _scatter_add(tgt, idx, src, axis=0):
    return tgt.at[idx].add(src)

def _segment_sum(src, seg, n):
    return jax.ops.segment_sum(src, seg, n)

class _Rng:

    def __init__(self, key):
        self._k = key

    def _next(self):
        self._k, sub = jax.random.split(self._k)
        return sub

    def normal(self, shape):
        return jax.random.normal(self._next(), shape, dtype=jnp.bfloat16)

    def randint(self, lo, hi, shape):
        return jax.random.randint(self._next(), shape, lo, hi, dtype=jnp.int32)

    def uniform(self, shape, lo=0.0, hi=1.0):
        return jax.random.uniform(self._next(), shape, jnp.bfloat16, lo, hi)

    def permutation(self, n):
        return jax.random.permutation(self._next(), n)
kernel_name = 'interleave_layers__memory_aug_infini_attn__mixer_s_mlp__prompt'

def setup_inputs():
    _rng = _Rng(jax.random.key(int.from_bytes(__import__("os").urandom(4), "little")))
    _w = lambda a: (lambda t: t.astype(jnp.bfloat16) if jnp.issubdtype(t.dtype, jnp.floating) else t)(jnp.asarray(a))

    def _A_setup():
        B, S, D, H = (1, 2048, 1024, 32)
        N = 4
        L = max(1, S // N)
        sc = D ** (-0.5)
        return {'x': _w((lambda *s: _rng.normal(s) * 0.05)(B, N * L, D)), 'wq': _w((lambda *s: _rng.normal(s) * 0.05)(D, D) * sc), 'wk': _w((lambda *s: _rng.normal(s) * 0.05)(D, D) * sc), 'wv': _w((lambda *s: _rng.normal(s) * 0.05)(D, D) * sc), 'wo': _w((lambda *s: _rng.normal(s) * 0.05)(D, D) * sc), 'beta': _w((lambda *s: _rng.normal(s) * 0.05)(H))}
    _A_in = _A_setup()

    def _B_setup():
        B, S, D, F = (1, 2048, 1024, 3584)
        return {'x': _w((lambda *s: _rng.normal(s) * 0.05)(B, S, D)), 'w1': _w((lambda *s: _rng.normal(s) * 0.05)(D, D) * D ** (-0.5)), 'w2': _w((lambda *s: _rng.normal(s) * 0.05)(D, D) * D ** (-0.5)), 'w3': _w((lambda *s: _rng.normal(s) * 0.05)(D, F) * D ** (-0.5)), 'w4': _w((lambda *s: _rng.normal(s) * 0.05)(F, D) * F ** (-0.5))}
    _B_in = _B_setup()
    return {'A_x': _A_in['x'], 'A_wq': _A_in['wq'], 'A_wk': _A_in['wk'], 'A_wv': _A_in['wv'], 'A_wo': _A_in['wo'], 'A_beta': _A_in['beta'], 'B_x': _B_in['x'], 'B_w1': _B_in['w1'], 'B_w2': _B_in['w2'], 'B_w3': _B_in['w3'], 'B_w4': _B_in['w4']}

def reference(A_x, A_wq, A_wk, A_wv, A_wo, A_beta, B_x, B_w1, B_w2, B_w3, B_w4):

    def _A_ref(x, wq, wk, wv, wo, beta):
        B, S, D = x.shape
        H = 32
        Dh = D // H
        N = 4
        L = S // N
        q = (lambda x, *d: x.transpose(*d))((x @ wq).reshape(B, S, H, Dh), 0, 2, 1, 3).reshape(B, H, N, L, Dh)
        k = (lambda x, *d: x.transpose(*d))((x @ wk).reshape(B, S, H, Dh), 0, 2, 1, 3).reshape(B, H, N, L, Dh)
        v = (lambda x, *d: x.transpose(*d))((x @ wv).reshape(B, S, H, Dh), 0, 2, 1, 3).reshape(B, H, N, L, Dh)
        phi = lambda t: jnp.where(t > 0, t + 1.0, jnp.exp(t))
        scale = Dh ** (-0.5)
        ar = jnp.arange(L)
        mask = (lambda x, dt: x.astype(dt))(ar[:, None] < ar[None, :], x.dtype) * -1000000000.0
        g = _sigmoid(beta).reshape(1, H, 1, 1)
        M = jnp.einsum('bhd,bhe->bhde', q[:, :, 0, 0, :] * 0.0, q[:, :, 0, 0, :] * 0.0)
        z = q[:, :, 0, 0, :] * 0.0
        outs = []
        for s in range(N):
            qs, ks, vs = (q[:, :, s].copy(), k[:, :, s].copy(), v[:, :, s].copy())
            logits = jnp.einsum('bhqd,bhkd->bhqk', qs, ks) * scale + mask
            p = _softmax(logits, axis=-1)
            a_dot = jnp.einsum('bhqk,bhkd->bhqd', p, vs)
            pq = phi(qs)
            num = jnp.einsum('bhld,bhde->bhle', pq, M)
            den = jnp.einsum('bhld,bhd->bhl', pq, z)[..., None] + 1e-06
            a_mem = num / den
            o = g * a_mem + (1.0 - g) * a_dot
            outs.append(o)
            pk = phi(ks)
            M = M + jnp.einsum('bhld,bhle->bhde', pk, vs)
            z = z + jnp.einsum('bhld->bhd', pk)
        o = (lambda x, *d: x.transpose(*d))(jnp.stack(outs, 2).reshape(B, H, S, Dh), 0, 2, 1, 3).reshape(B, S, D)
        return o @ wo

    def _B_ref(x, w1, w2, w3, w4):
        B, S, D = x.shape
        h = _gelu(_layernorm(x, axis=-1) @ w1)
        c = D // 4
        g0 = jnp.pad(h[:, :, 0 * c:1 * c], ((0, 0), (1, 0), (0, 0)))[:, :S, :]
        g1 = jnp.pad(h[:, :, 1 * c:2 * c], ((0, 0), (0, 1), (0, 0)))[:, 1:, :]
        g2 = jnp.pad(h[:, :, 2 * c:3 * c], ((0, 0), (2, 0), (0, 0)))[:, :S, :]
        g3 = jnp.pad(h[:, :, 3 * c:], ((0, 0), (0, 2), (0, 0)))[:, 2:, :]
        hs = jnp.concatenate([g0, g1, g2, g3], axis=-1) @ w2
        x1 = x + hs
        h2 = _gelu(_layernorm(x1, axis=-1) @ w3) @ w4
        return x1 + h2
    x = A_x
    x = x + _A_ref(_layernorm(x, axis=-1), A_wq, A_wk, A_wv, A_wo, A_beta)
    x = x + _B_ref(_layernorm(x, axis=-1), B_w1, B_w2, B_w3, B_w4)
    x = x + _A_ref(_layernorm(x, axis=-1), A_wq, A_wk, A_wv, A_wo, A_beta)
    x = x + _B_ref(_layernorm(x, axis=-1), B_w1, B_w2, B_w3, B_w4)
    return x
```

```python
import math

import jax
import jax.numpy as jnp
import jax.experimental.pallas as pl
import jax.experimental.pallas.tpu as pltpu

S, D, H, F = 2048, 1024, 32, 3584
DH = D // H
NSEG = 4
L = S // NSEG
NG = D // 128
HPG = 128 // DH
EPS = 1e-5
LOG2E = 1.4426950408889634
F32 = jnp.float32
BF16 = jnp.bfloat16
FC = 512


def _ln(x):
    m = jnp.mean(x, axis=-1, keepdims=True)
    xc = x - m
    v = jnp.mean(xc * xc, axis=-1, keepdims=True)
    return xc * jax.lax.rsqrt(v + EPS)


def _gelu(x):
    c = math.sqrt(2.0 / math.pi)
    return 0.5 * x * (1.0 + jnp.tanh(c * (x + 0.044715 * (x * x * x))))


def _phi(t):
    return jnp.where(t > 0, t + 1.0, jnp.exp(t))


def _dot(a, b):
    return jnp.dot(a, b, preferred_element_type=F32)


def _dot_nt(a, b):
    return jax.lax.dot_general(a, b, (((1,), (1,)), ((), ())), preferred_element_type=F32)


def _dot_tn(a, b):
    return jax.lax.dot_general(a, b, (((0,), (0,)), ((), ())), preferred_element_type=F32)


def _kernel(x_hbm, wq_hbm, wk_hbm, wv_hbm, wo_hbm, beta_ref, w1_hbm, w2_hbm, w3_hbm, w4_hbm,
            out_hbm,
            xin, xres, wq, wk, wv, wo, w1, w2, w3, w4,
            qs_s, pq_s, k_s, pk_s, v_s, o_s, m_s, z_s, g_s, y_s, h_s, ob_s, sems, osems):
    copies = [pltpu.make_async_copy(src, dst, sems.at[i]) for i, (src, dst) in enumerate([
        (x_hbm, xin), (wq_hbm, wq), (wk_hbm, wk), (wv_hbm, wv), (wo_hbm, wo),
        (w1_hbm, w1), (w2_hbm, w2), (w3_hbm, w3), (w4_hbm, w4)])]
    for c in copies:
        c.start()

    gate = jax.nn.sigmoid(beta_ref[...].astype(F32))
    hid = jax.lax.broadcasted_iota(jnp.int32, (1, 128), 1)
    lane128 = jax.lax.broadcasted_iota(jnp.int32, (1, 128), 1) // DH
    for g in range(NG):
        row = jnp.zeros((1, 128), F32)
        for h in range(HPG):
            val = jnp.sum(jnp.where(hid == g * HPG + h, gate, 0.0), axis=1, keepdims=True)
            row = jnp.where(lane128 == h, val, row)
        g_s[g] = jnp.broadcast_to(row, (8, 128))

    h_s[pl.ds(0, 8), :] = jnp.zeros((8, D), F32)
    h_s[pl.ds(S + 8, 8), :] = jnp.zeros((8, D), F32)

    copies[0].wait()

    def init_body(b, c):
        r0 = pl.multiple_of(b * L, L)
        xres[pl.ds(r0, L), :] = xin[pl.ds(r0, L), :].astype(F32)
        return c
    jax.lax.fori_loop(0, NSEG, init_body, 0)

    scale = DH ** -0.5
    lane_head = jax.lax.broadcasted_iota(jnp.int32, (128, 128), 1) // DH
    row_head = jax.lax.broadcasted_iota(jnp.int32, (128, 128), 0) // DH

    def rep_body(rep, carry):
        @pl.when(rep == 0)
        def _():
            for c in copies[1:5]:
                c.wait()

        m_s[...] = jnp.zeros(m_s.shape, F32)
        z_s[...] = jnp.zeros(z_s.shape, F32)

        def seg_body(s, c):
            r0 = pl.multiple_of(s * L, L)
            xs = xres[pl.ds(r0, L), :]
            xn = _ln(xs).astype(BF16)
            q = _dot(xn, wq[...])
            k = _dot(xn, wk[...])
            v = _dot(xn, wv[...])
            qs = (q * (scale * LOG2E)).astype(BF16)
            pq = _phi(q).astype(BF16)
            kb = k.astype(BF16)
            pk = _phi(k).astype(BF16)
            vb = v.astype(BF16)
            for g in range(NG):
                sl = slice(g * 128, (g + 1) * 128)
                qs_s[g] = qs[:, sl]
                pq_s[g] = pq[:, sl]
                k_s[g] = kb[:, sl]
                pk_s[g] = pk[:, sl]
                v_s[g] = vb[:, sl]

            def grp_body(g, c2):
                qg = qs_s[g]
                kg = k_s[g]
                vg = v_s[g]
                pqg = pq_s[g]
                pkg = pk_s[g]
                gv = g_s[g][0:1, :]
                bd = lane_head == row_head
                mg = m_s[g]
                zrow = z_s[g][0:1, :]
                num = _dot(pqg, mg.astype(BF16))
                bones = jnp.where(bd, 1.0, 0.0).astype(BF16)
                den = _dot((pqg.astype(F32) * zrow).astype(BF16), bones) + 1e-6
                amem = num / den
                upd = _dot_tn(pkg, vg)
                m_s[g] = mg + jnp.where(bd, upd, 0.0)
                z_s[g] = z_s[g] + jnp.sum(pkg.astype(F32), axis=0, keepdims=True)
                rr = jax.lax.broadcasted_iota(jnp.int32, (HPG * 128, 128), 0) % 128
                cc = jax.lax.broadcasted_iota(jnp.int32, (HPG * 128, 128), 1)
                madd = jnp.where(rr < cc, -1e9 * LOG2E, 0.0).astype(F32)
                for i in range(4):
                    qi = qg[i * 128:(i + 1) * 128]
                    qst = jnp.concatenate(
                        [jnp.where(lane_head == h, qi, jnp.zeros_like(qi)) for h in range(HPG)], axis=0)
                    nk = (i + 1) * 128
                    sd = _dot_nt(qst, kg[i * 128:nk]) + madd
                    if i > 0:
                        so = _dot_nt(qst, kg[0:i * 128])
                        sc = jnp.concatenate([so, sd], axis=1)
                    else:
                        sc = sd
                    mx = jnp.max(sc, axis=1, keepdims=True)
                    p = jnp.exp2(sc - mx)
                    lsum = jnp.sum(p, axis=1, keepdims=True)
                    o = _dot(p.astype(BF16), vg[0:nk]) / lsum
                    od = o[0:128]
                    for h in range(1, HPG):
                        od = jnp.where(lane_head == h, o[h * 128:(h + 1) * 128], od)
                    res = gv * amem[i * 128:(i + 1) * 128] + (1.0 - gv) * od
                    o_s[g, pl.ds(i * 128, 128), :] = res.astype(BF16)
                return c2
            jax.lax.fori_loop(0, NG, grp_body, 0)

            ocat = jnp.concatenate([o_s[g] for g in range(NG)], axis=1)
            xres[pl.ds(r0, L), :] = xs + _dot(ocat, wo[...])
            return c
        jax.lax.fori_loop(0, NSEG, seg_body, 0)

        @pl.when(rep == 0)
        def _():
            for c in copies[5:7]:
                c.wait()

        def b1_body(b, c):
            r0 = pl.multiple_of(b * L, L)
            y = _ln(xres[pl.ds(r0, L), :])
            y_s[pl.ds(r0, L), :] = y
            h = _gelu(_dot(_ln(y).astype(BF16), w1[...]))
            h_s[pl.ds(r0 + 8, L), :] = h
            return c
        jax.lax.fori_loop(0, NSEG, b1_body, 0)

        @pl.when(rep == 0)
        def _():
            for c in copies[7:9]:
                c.wait()

        def b2_body(b, c):
            r0 = pl.multiple_of(b * L, L)
            cw = D // 4
            hsh = jnp.concatenate([
                h_s[pl.ds(r0, L + 16), i * cw:(i + 1) * cw][8 + sh:8 + sh + L]
                for i, sh in enumerate((-1, 1, -2, 2))], axis=1).astype(BF16)
            x1 = y_s[pl.ds(r0, L), :] + _dot(hsh, w2[...])
            u = _ln(x1).astype(BF16)
            acc = xres[pl.ds(r0, L), :] + x1
            for f in range(F // FC):
                a = _gelu(_dot(u, w3[:, f * FC:(f + 1) * FC])).astype(BF16)
                acc = acc + _dot(a, w4[f * FC:(f + 1) * FC, :])
            xres[pl.ds(r0, L), :] = acc

            @pl.when(rep == 1)
            def _():
                ob_s[pl.ds(r0, L), :] = acc.astype(BF16)
                pltpu.make_async_copy(ob_s.at[pl.ds(r0, L), :], out_hbm.at[pl.ds(r0, L), :],
                                      osems.at[b]).start()
            return c
        jax.lax.fori_loop(0, NSEG, b2_body, 0)
        return carry

    jax.lax.fori_loop(0, 2, rep_body, 0)

    for b in range(NSEG):
        pltpu.make_async_copy(ob_s.at[pl.ds(b * L, L), :], out_hbm.at[pl.ds(b * L, L), :],
                              osems.at[b]).wait()


@jax.jit
def pallas_interleave_layers__memory_aug_infini_attn__mixer_s_mlp__prompt_kernel(
    A_x, A_wq, A_wk, A_wv, A_wo, A_beta, B_x, B_w1, B_w2, B_w3, B_w4,
):
    x = A_x.reshape(S, D)
    beta = jnp.pad(A_beta.reshape(1, H), ((0, 0), (0, 128 - H)))
    anyspec = pl.BlockSpec(memory_space=pl.ANY)
    scratch = [
        pltpu.VMEM((S, D), BF16),
        pltpu.VMEM((S, D), F32),
        pltpu.VMEM((D, D), BF16), pltpu.VMEM((D, D), BF16), pltpu.VMEM((D, D), BF16),
        pltpu.VMEM((D, D), BF16), pltpu.VMEM((D, D), BF16), pltpu.VMEM((D, D), BF16),
        pltpu.VMEM((D, F), BF16), pltpu.VMEM((F, D), BF16),
        pltpu.VMEM((NG, L, 128), BF16), pltpu.VMEM((NG, L, 128), BF16), pltpu.VMEM((NG, L, 128), BF16),
        pltpu.VMEM((NG, L, 128), BF16), pltpu.VMEM((NG, L, 128), BF16), pltpu.VMEM((NG, L, 128), BF16),
        pltpu.VMEM((NG, 128, 128), F32),
        pltpu.VMEM((NG, 8, 128), F32),
        pltpu.VMEM((NG, 8, 128), F32),
        pltpu.VMEM((S, D), F32),
        pltpu.VMEM((S + 16, D), F32),
        pltpu.VMEM((S, D), BF16),
        pltpu.SemaphoreType.DMA((9,)),
        pltpu.SemaphoreType.DMA((NSEG,)),
    ]
    out = pl.pallas_call(
        _kernel,
        out_shape=jax.ShapeDtypeStruct((S, D), BF16),
        in_specs=[anyspec] * 5 + [pl.BlockSpec(memory_space=pltpu.VMEM)] + [anyspec] * 4,
        out_specs=anyspec,
        scratch_shapes=scratch,
        compiler_params=pltpu.CompilerParams(vmem_limit_bytes=110 * 1024 * 1024),
    )(x, A_wq, A_wk, A_wv, A_wo, beta, B_w1, B_w2, B_w3, B_w4)
    return out.reshape(1, S, D)
```

```python
import math

import jax
import jax.numpy as jnp
import jax.experimental.pallas as pl
import jax.experimental.pallas.tpu as pltpu

S, D, H, F = 2048, 1024, 32, 3584
DH = D // H
NSEG = 4
L = S // NSEG
NG = D // 128
HPG = 128 // DH
EPS = 1e-5
LOG2E = 1.4426950408889634
F32 = jnp.float32
BF16 = jnp.bfloat16
FC = 512
NFA = 3
SCOPES = False


class _NoScope:
    def __enter__(self):
        return self

    def __exit__(self, *a):
        return False


def _scope(name):
    return jax.named_scope(name) if SCOPES else _NoScope()


def _ln(x):
    m = jnp.mean(x, axis=-1, keepdims=True)
    xc = x - m
    v = jnp.mean(xc * xc, axis=-1, keepdims=True)
    return xc * jax.lax.rsqrt(v + EPS)


def _gelu(x):
    c = math.sqrt(2.0 / math.pi)
    hx = 0.5 * x
    return hx + hx * jnp.tanh(x * (c + (c * 0.044715) * (x * x)))


def _phi(t):
    return jnp.where(t > 0, t + 1.0, jnp.exp(t))


def _dot(a, b):
    return jnp.dot(a, b, preferred_element_type=F32)


def _dot_nt(a, b):
    return jax.lax.dot_general(a, b, (((1,), (1,)), ((), ())), preferred_element_type=F32)


def _kernel(x_hbm, wq_hbm, wk_hbm, wv_hbm, wo_hbm, beta_ref, w1_hbm, w2_hbm, w3_hbm, w4_hbm,
            out_hbm,
            xin, xres, wq, wk, wv, wo, w1, w2, w3, w4,
            qs_s, pq_s, k_s, pk_s, vt_s, o_s, m_s, z_s, g_s, y_s, h_s, u_s, ob_s, xsems, sems, osems):
    xcopies = [pltpu.make_async_copy(x_hbm.at[pl.ds(b * L, L), :], xin.at[pl.ds(b * L, L), :], xsems.at[b])
               for b in range(NSEG)]
    copies = [pltpu.make_async_copy(src, dst, sems.at[i]) for i, (src, dst) in enumerate([
        (wq_hbm, wq), (wk_hbm, wk), (wv_hbm, wv), (wo_hbm, wo),
        (w1_hbm, w1), (w2_hbm, w2), (w3_hbm, w3), (w4_hbm, w4)])]
    xcopies[0].start()
    for c in copies[0:3]:
        c.start()
    for c in xcopies[1:]:
        c.start()
    for c in copies[3:]:
        c.start()

    gate = jax.nn.sigmoid(beta_ref[...].astype(F32))
    hid = jax.lax.broadcasted_iota(jnp.int32, (128, 128), 1)
    rid = jax.lax.broadcasted_iota(jnp.int32, (128, 128), 0) // DH
    rsel = jax.lax.broadcasted_iota(jnp.int32, (128, 1), 0) // DH
    for g in range(NG):
        col = jnp.sum(jnp.where(hid == g * HPG + rid, gate, 0.0), axis=1, keepdims=True)
        g_s[g] = jnp.broadcast_to(col, (128, 128))

    h_s[pl.ds(0, 8), :] = jnp.zeros((8, D), F32)
    h_s[pl.ds(S + 8, 8), :] = jnp.zeros((8, D), F32)

    scale = DH ** -0.5
    lane_head = jax.lax.broadcasted_iota(jnp.int32, (128, 128), 1) // DH
    row_head = jax.lax.broadcasted_iota(jnp.int32, (128, 128), 0) // DH

    def rep_body(rep, carry):
        m_s[...] = jnp.zeros(m_s.shape, F32)
        z_s[...] = jnp.zeros(z_s.shape, F32)

        def seg_body(s, c):
            r0 = pl.multiple_of(s * L, L)

            @pl.when(rep == 0)
            def _():
                pltpu.make_async_copy(x_hbm.at[pl.ds(r0, L), :], xin.at[pl.ds(r0, L), :], xsems.at[s]).wait()
                xres[pl.ds(r0, L), :] = xin[pl.ds(r0, L), :].astype(F32)

                @pl.when(s == 0)
                def _():
                    for cp in copies[0:3]:
                        cp.wait()

            with _scope('qkv'):
                xs = xres[pl.ds(r0, L), :]
                xn = _ln(xs).astype(BF16)
                q = _dot(xn, wq[...])
                k = _dot(xn, wk[...])
                v = _dot(xn, wv[...])
                qs = (q * (scale * LOG2E)).astype(BF16)
                pq = _phi(q).astype(BF16)
                kb = k.astype(BF16)
                pk = _phi(k).astype(BF16)
                for g in range(NG):
                    sl = slice(g * 128, (g + 1) * 128)
                    qs_s[g] = qs[:, sl]
                    pq_s[g] = pq[:, sl]
                    k_s[g] = kb[:, sl]
                    pk_s[g] = pk[:, sl]
                    vt_s[g] = v[:, sl].T.astype(BF16)

            def grp_body(g, c2):
                qg = qs_s[g]
                kg = k_s[g]
                vtg = vt_s[g]
                pqg = pq_s[g]
                pkg = pk_s[g]
                gt = g_s[g]
                bd = lane_head == row_head
                mg = m_s[g]
                zrow = z_s[g][0:1, :]
                z16 = jnp.where(jax.lax.broadcasted_iota(jnp.int32, (16, 128), 0)
                                == jax.lax.broadcasted_iota(jnp.int32, (16, 128), 1) // DH, zrow, 0.0)
                lhs = jnp.concatenate([mg, z16], axis=0).astype(BF16)
                nd = _dot_nt(lhs, pqg)
                rden = 1.0 / (nd[128:136] + 1e-6)
                upd = _dot(vtg, pkg)
                m_s[g] = mg + jnp.where(bd, upd, 0.0)
                z_s[g] = z_s[g] + jnp.sum(pkg.astype(F32), axis=0, keepdims=True)
                rr = jax.lax.broadcasted_iota(jnp.int32, (128, 128), 0)
                cc = jax.lax.broadcasted_iota(jnp.int32, (128, 128), 1)
                madd = jnp.where(cc < rr, -1e9 * LOG2E, 0.0).astype(F32)
                qgu = pltpu.bitcast(qg, jnp.uint32)
                hmask = [jnp.where(jax.lax.broadcasted_iota(jnp.int32, (64, 128), 1) // DH == h,
                                   jnp.uint32(0xFFFFFFFF), jnp.uint32(0)) for h in range(HPG)]
                madd4 = jnp.concatenate([madd] * HPG, axis=1)
                for i in range(4):
                    nk = (i + 1) * 128
                    qiu = qgu[i * 64:(i + 1) * 64]
                    qst = jnp.concatenate([pltpu.bitcast(qiu & hmask[h], BF16) for h in range(HPG)], axis=0)
                    sd = _dot_nt(kg[i * 128:nk], qst) + madd4
                    if i > 0:
                        so = _dot_nt(kg[0:i * 128], qst)
                        st = jnp.concatenate([so, sd], axis=0)
                    else:
                        st = sd
                    mx = jnp.max(st, axis=0, keepdims=True)
                    p = jnp.exp2(st - mx)
                    rl = 1.0 / jnp.sum(p, axis=0, keepdims=True)
                    pb = p.astype(BF16)
                    ots = []
                    for h in range(HPG):
                        hs = slice(h * 128, (h + 1) * 128)
                        ot = _dot(vtg[h * DH:(h + 1) * DH, 0:nk], pb[:, hs])
                        am = nd[h * DH:(h + 1) * DH, i * 128:nk] * rden[h:h + 1, i * 128:nk]
                        gh = gt[h * DH:(h + 1) * DH]
                        ots.append(gh * am + (1.0 - gh) * (ot * rl[:, hs]))
                    res = jnp.concatenate(ots, axis=0)
                    o_s[g, pl.ds(i * 128, 128), :] = res.T.astype(BF16)
                return c2
            with _scope('attn'):
                jax.lax.fori_loop(0, NG, grp_body, 0)

            @pl.when(jnp.logical_and(rep == 0, s == 0))
            def _():
                copies[3].wait()

            with _scope('oproj'):
                ocat = jnp.concatenate([o_s[g] for g in range(NG)], axis=1)
                xres[pl.ds(r0, L), :] = xs + _dot(ocat, wo[...])
            return c
        with _scope('layerA'):
            jax.lax.fori_loop(0, NSEG, seg_body, 0)

        @pl.when(rep == 0)
        def _():
            for cp in copies[4:6]:
                cp.wait()

        def b1_body(b, c):
            r0 = pl.multiple_of(b * L, L)
            y = _ln(xres[pl.ds(r0, L), :])
            y_s[pl.ds(r0, L), :] = y
            h = _gelu(_dot(_ln(y).astype(BF16), w1[...]))
            h_s[pl.ds(r0 + 8, L), :] = h
            return c
        with _scope('B1'):
            jax.lax.fori_loop(0, NSEG, b1_body, 0)

        @pl.when(rep == 0)
        def _():
            for cp in copies[6:8]:
                cp.wait()

        def b2a_body(b, c):
            r0 = pl.multiple_of(b * L, L)
            cw = D // 4
            hsh = jnp.concatenate([
                h_s[pl.ds(r0, L + 16), i * cw:(i + 1) * cw][8 + sh:8 + sh + L]
                for i, sh in enumerate((-1, 1, -2, 2))], axis=1).astype(BF16)
            x1 = y_s[pl.ds(r0, L), :] + _dot(hsh, w2[...])
            u = _ln(x1).astype(BF16)
            u_s[pl.ds(r0, L), :] = u
            acc = xres[pl.ds(r0, L), :] + x1
            for f in range(NFA):
                a = _gelu(_dot(u, w3[:, f * FC:(f + 1) * FC])).astype(BF16)
                acc = acc + _dot(a, w4[f * FC:(f + 1) * FC, :])
            xres[pl.ds(r0, L), :] = acc
            return c
        with _scope('B2a'):
            jax.lax.fori_loop(0, NSEG, b2a_body, 0)

        def b2b_body(b, c):
            r0 = pl.multiple_of(b * L, L)
            u = u_s[pl.ds(r0, L), :]
            acc = xres[pl.ds(r0, L), :]
            for f in range(NFA, F // FC):
                a = _gelu(_dot(u, w3[:, f * FC:(f + 1) * FC])).astype(BF16)
                acc = acc + _dot(a, w4[f * FC:(f + 1) * FC, :])
            xres[pl.ds(r0, L), :] = acc

            @pl.when(rep == 1)
            def _():
                ob_s[pl.ds(r0, L), :] = acc.astype(BF16)
                pltpu.make_async_copy(ob_s.at[pl.ds(r0, L), :], out_hbm.at[pl.ds(r0, L), :],
                                      osems.at[b]).start()
            return c
        with _scope('B2b'):
            jax.lax.fori_loop(0, NSEG, b2b_body, 0)
        return carry

    jax.lax.fori_loop(0, 2, rep_body, 0)

    for b in range(NSEG):
        pltpu.make_async_copy(ob_s.at[pl.ds(b * L, L), :], out_hbm.at[pl.ds(b * L, L), :],
                              osems.at[b]).wait()


@jax.jit
def pallas_interleave_layers__memory_aug_infini_attn__mixer_s_mlp__prompt_kernel(
    A_x, A_wq, A_wk, A_wv, A_wo, A_beta, B_x, B_w1, B_w2, B_w3, B_w4,
):
    x = A_x.reshape(S, D)
    beta = jnp.pad(A_beta.reshape(1, H), ((0, 0), (0, 128 - H)))
    anyspec = pl.BlockSpec(memory_space=pl.ANY)
    scratch = [
        pltpu.VMEM((S, D), BF16),
        pltpu.VMEM((S, D), F32),
        pltpu.VMEM((D, D), BF16), pltpu.VMEM((D, D), BF16), pltpu.VMEM((D, D), BF16),
        pltpu.VMEM((D, D), BF16), pltpu.VMEM((D, D), BF16), pltpu.VMEM((D, D), BF16),
        pltpu.VMEM((D, F), BF16), pltpu.VMEM((F, D), BF16),
        pltpu.VMEM((NG, L, 128), BF16), pltpu.VMEM((NG, L, 128), BF16), pltpu.VMEM((NG, L, 128), BF16),
        pltpu.VMEM((NG, L, 128), BF16),
        pltpu.VMEM((NG, 128, L), BF16),
        pltpu.VMEM((NG, L, 128), BF16),
        pltpu.VMEM((NG, 128, 128), F32),
        pltpu.VMEM((NG, 8, 128), F32),
        pltpu.VMEM((NG, 128, 128), F32),
        pltpu.VMEM((S, D), F32),
        pltpu.VMEM((S + 16, D), F32),
        pltpu.VMEM((S, D), BF16),
        pltpu.VMEM((S, D), BF16),
        pltpu.SemaphoreType.DMA((NSEG,)),
        pltpu.SemaphoreType.DMA((8,)),
        pltpu.SemaphoreType.DMA((NSEG,)),
    ]
    out = pl.pallas_call(
        _kernel,
        out_shape=jax.ShapeDtypeStruct((S, D), BF16),
        in_specs=[anyspec] * 5 + [pl.BlockSpec(memory_space=pltpu.VMEM)] + [anyspec] * 4,
        out_specs=anyspec,
        scratch_shapes=scratch,
        compiler_params=pltpu.CompilerParams(vmem_limit_bytes=110 * 1024 * 1024),
    )(x, A_wq, A_wk, A_wv, A_wo, beta, B_w1, B_w2, B_w3, B_w4)
    return out.reshape(1, S, D)
```

```python
import math

import jax
import jax.numpy as jnp
import jax.experimental.pallas as pl
import jax.experimental.pallas.tpu as pltpu

S, D, H, F = 2048, 1024, 32, 3584
DH = D // H
NSEG = 4
L = S // NSEG
NG = D // 128
HPG = 128 // DH
EPS = 1e-5
LOG2E = 1.4426950408889634
F32 = jnp.float32
BF16 = jnp.bfloat16
FC = 512
NFA = 3
SCOPES = False
GU = 8
ORDER = (0, 1, 2, 3)
SPLIT_QKV = 2
SPLIT_OB = 4
SPLIT_B2 = 2
OB_MODE = 0
B2_MODE = 0
L_LO = 2.0 ** -30
L_HI = 2.0 ** 30


class _NoScope:
    def __enter__(self):
        return self

    def __exit__(self, *a):
        return False


def _scope(name):
    return jax.named_scope(name) if SCOPES else _NoScope()


def _lane0(g):
    return g * 128 if isinstance(g, int) else pl.multiple_of(g * 128, 128)


def _ln(x):
    m = jnp.mean(x, axis=-1, keepdims=True)
    xc = x - m
    v = jnp.mean(xc * xc, axis=-1, keepdims=True)
    return xc * jax.lax.rsqrt(v + EPS)


def _gelu(x):
    c = math.sqrt(2.0 / math.pi)
    hx = 0.5 * x
    return hx + hx * jnp.tanh(x * (c + (c * 0.044715) * (x * x)))


def _phi(t):
    return jnp.where(t > 0, t + 1.0, jnp.exp(t))


def _dot(a, b):
    return jnp.dot(a, b, preferred_element_type=F32)


def _dot_nt(a, b):
    return jax.lax.dot_general(a, b, (((1,), (1,)), ((), ())), preferred_element_type=F32)


def _kernel(x_hbm, wq_hbm, wk_hbm, wv_hbm, wo_hbm, beta_ref, w1_hbm, w2_hbm, w3_hbm, w4_hbm,
            out_hbm,
            xin, xres, xb_s, xc_s, wq, wk, wv, wo, w1, w2, w3, w4,
            qs_s, pq_s, k_s, pk_s, vt_s, o_s, m_s, z_s, g_s, y_s, h_s, u_s, xsems, sems, osems):
    xcopies = [pltpu.make_async_copy(x_hbm.at[pl.ds(b * L, L), :], xin.at[pl.ds(b * L, L), :], xsems.at[b])
               for b in range(NSEG)]
    copies = [pltpu.make_async_copy(src, dst, sems.at[i]) for i, (src, dst) in enumerate([
        (wq_hbm, wq), (wk_hbm, wk), (wv_hbm, wv), (wo_hbm, wo),
        (w1_hbm, w1), (w2_hbm, w2), (w3_hbm, w3), (w4_hbm, w4)])]
    xcopies[0].start()
    for c in copies[0:3]:
        c.start()

    gate = jax.nn.sigmoid(beta_ref[...].astype(F32))
    hid = jax.lax.broadcasted_iota(jnp.int32, (128, 128), 1)
    rid = jax.lax.broadcasted_iota(jnp.int32, (128, 128), 0) // DH
    for g in range(NG):
        col = jnp.sum(jnp.where(hid == g * HPG + rid, gate, 0.0), axis=1, keepdims=True)
        g_s[g] = jnp.broadcast_to(col, (128, 128))

    h_s[pl.ds(0, 8), :] = jnp.zeros((8, D), F32)
    h_s[pl.ds(S + 8, 8), :] = jnp.zeros((8, D), F32)

    scale = DH ** -0.5

    def attention(s, par, truemax, gu, bad0):
        def grp_body(gi, bad):
            bd = (jax.lax.broadcasted_iota(jnp.int32, (128, 128), 1) // DH
                  == jax.lax.broadcasted_iota(jnp.int32, (128, 128), 0) // DH)
            rr = jax.lax.broadcasted_iota(jnp.int32, (128, 128), 0)
            cc = jax.lax.broadcasted_iota(jnp.int32, (128, 128), 1)
            madd = jnp.where(cc < rr, -1e9 * LOG2E, 0.0).astype(F32)
            madd4 = jnp.concatenate([madd] * HPG, axis=1)
            hmask = [jnp.where(jax.lax.broadcasted_iota(jnp.int32, (64, 128), 1) // DH == h,
                               jnp.uint32(0xFFFFFFFF), jnp.uint32(0)) for h in range(HPG)]

            def mem(g):
                pqg = pq_s[s, g]
                pkg = pk_s[s, g]
                mg = m_s[par, g]
                zv = z_s[par, g]
                z16 = jnp.where(jax.lax.broadcasted_iota(jnp.int32, (16, 128), 0)
                                == jax.lax.broadcasted_iota(jnp.int32, (16, 128), 1) // DH, zv[0:1, :], 0.0)
                lhs = jnp.concatenate([mg, z16], axis=0).astype(BF16)
                nd = _dot_nt(lhs, pqg)
                rden = 1.0 / (nd[128:136] + 1e-6)
                if not truemax:
                    upd = _dot(vt_s[s, g], pkg)
                    m_s[1 - par, g] = mg + jnp.where(bd, upd, 0.0)
                    z_s[1 - par, g] = zv + jnp.sum(pkg.astype(F32), axis=0, keepdims=True)
                return nd, rden

            def qk(g, i):
                qiu = pltpu.bitcast(qs_s[s, g, pl.ds(i * 128, 128), :], jnp.uint32)
                qst = jnp.concatenate([pltpu.bitcast(qiu & hmask[h], BF16) for h in range(HPG)], axis=0)
                sd = _dot_nt(k_s[s, g, pl.ds(i * 128, 128), :], qst) + madd4
                if i > 0:
                    so = _dot_nt(k_s[s, g, pl.ds(0, i * 128), :], qst)
                    return jnp.concatenate([so, sd], axis=0)
                return sd

            def sm(st):
                if truemax:
                    p = jnp.exp2(st - jnp.max(st, axis=0, keepdims=True))
                else:
                    p = jnp.exp2(st)
                lsum = jnp.sum(p, axis=0, keepdims=True)
                return [p[:, h * 128:(h + 1) * 128].astype(BF16) for h in range(HPG)], lsum

            def pv(g, i, pbs, rl, nd, rden):
                nk = (i + 1) * 128
                ots = []
                for h in range(HPG):
                    hs = slice(h * 128, (h + 1) * 128)
                    ot = _dot(vt_s[s, g, pl.ds(h * DH, DH), pl.ds(0, nk)], pbs[h])
                    am = nd[h * DH:(h + 1) * DH, i * 128:nk] * rden[h:h + 1, i * 128:nk]
                    gh = g_s[g, pl.ds(h * DH, DH), :]
                    ots.append(gh * am + (1.0 - gh) * (ot * rl[:, hs]))
                res = jnp.concatenate(ots, axis=0)
                o_s[pl.ds(i * 128, 128), pl.ds(_lane0(g), 128)] = res.T.astype(BF16)

            gs = [gi * gu + u for u in range(gu)]
            stages = [(u, i) for u in range(gu) for i in ORDER]
            mems = {}
            sts = {stages[0]: qk(gs[stages[0][0]], stages[0][1])}
            for n, (u, i) in enumerate(stages):
                if u not in mems:
                    mems[u] = mem(gs[u])
                if n + 1 < len(stages):
                    u2, i2 = stages[n + 1]
                    sts[stages[n + 1]] = qk(gs[u2], i2)
                pbs, lsum = sm(sts.pop((u, i)))
                if not truemax:
                    ok = jnp.logical_and(lsum >= L_LO, lsum <= L_HI)
                    bad = jnp.where(ok, bad, 1.0)
                pv(gs[u], i, pbs, 1.0 / lsum, *mems[u])
            return bad
        return jax.lax.fori_loop(0, NG // gu, grp_body, bad0)

    def rep_body(rep, carry):
        def qkv_body(s, c):
            r0 = pl.multiple_of(s * L, L)

            @pl.when(rep == 0)
            def _():
                pltpu.make_async_copy(x_hbm.at[pl.ds(r0, L), :], xin.at[pl.ds(r0, L), :], xsems.at[s]).wait()
                xres[pl.ds(r0, L), :] = xin[pl.ds(r0, L), :].astype(F32)

                @pl.when(s == 0)
                def _():
                    for cp in copies[0:3]:
                        cp.wait()
                    for cp in xcopies[1:] + copies[3:]:
                        cp.start()

            n = SPLIT_QKV
            hr = L // n
            xns = [_ln(xres[pl.ds(r0 + j * hr, hr), :]).astype(BF16) for j in range(n)]
            for j in range(n):
                rows = pl.ds(j * hr, hr)
                xn = xns[j]
                q = _dot(xn, wq[...])
                k = _dot(xn, wk[...])
                v = _dot(xn, wv[...])
                qs = (q * (scale * LOG2E)).astype(BF16)
                pq = _phi(q).astype(BF16)
                kb = k.astype(BF16)
                pk = _phi(k).astype(BF16)
                for g in range(NG):
                    sl = slice(g * 128, (g + 1) * 128)
                    qs_s[s, g, rows, :] = qs[:, sl]
                    pq_s[s, g, rows, :] = pq[:, sl]
                    k_s[s, g, rows, :] = kb[:, sl]
                    pk_s[s, g, rows, :] = pk[:, sl]
                    vt_s[s, g, :, rows] = v[:, sl].T.astype(BF16)
            return c
        with _scope('qkv'):
            jax.lax.fori_loop(0, NSEG, qkv_body, 0)

        m_s[0] = jnp.zeros(m_s.shape[1:], F32)
        z_s[0] = jnp.zeros(z_s.shape[1:], F32)

        def seg_body(s, c):
            r0 = pl.multiple_of(s * L, L)
            par = s % 2
            with _scope('attn'):
                bad = attention(s, par, False, GU, jnp.zeros((1, HPG * 128), F32))

            @pl.when(jnp.max(bad) > 0.0)
            def _():
                attention(s, par, True, 1, jnp.zeros((1, HPG * 128), F32))

            @pl.when(jnp.logical_and(rep == 0, s == 0))
            def _():
                copies[3].wait()
                copies[4].wait()

            with _scope('ob1'):
                n = SPLIT_OB
                hr = L // n

                def oproj(j):
                    ocat = o_s[pl.ds(j * hr, hr), :]
                    return xres[pl.ds(r0 + j * hr, hr), :] + _dot(ocat, wo[...])

                def lns(j, xj):
                    rows = pl.ds(r0 + j * hr, hr)
                    xb_s[rows, :] = xj
                    y = _ln(xj)
                    y_s[rows, :] = y
                    return _ln(y).astype(BF16)

                def w1g(j, yn):
                    h_s[pl.ds(r0 + 8 + j * hr, hr), :] = _gelu(_dot(yn, w1[...]))

                if OB_MODE == 0:
                    xs = [oproj(j) for j in range(n)]
                    for j in range(n):
                        w1g(j, lns(j, xs[j]))
                elif OB_MODE == 1:
                    nxt = oproj(0)
                    for j in range(n):
                        cur = nxt
                        if j + 1 < n:
                            nxt = oproj(j + 1)
                        w1g(j, lns(j, cur))
                elif OB_MODE == 2:
                    xs = [oproj(j) for j in range(n)]
                    yns = [lns(j, xs[j]) for j in range(n)]
                    for j in range(n):
                        w1g(j, yns[j])
                elif OB_MODE == 3:
                    xs = [oproj(0), oproj(1)]
                    yns = []
                    for j in range(n):
                        if j + 2 < n:
                            xs.append(oproj(j + 2))
                        yns.append(lns(j, xs[j]))
                        if j >= 1:
                            w1g(j - 1, yns[j - 1])
                    w1g(n - 1, yns[n - 1])
            return c
        with _scope('seg'):
            jax.lax.fori_loop(0, NSEG, seg_body, 0)

        @pl.when(rep == 0)
        def _():
            for cp in copies[5:8]:
                cp.wait()

        def b2a_body(b, c):
            r0 = pl.multiple_of(b * L, L)
            cw = D // 4
            n = SPLIT_B2
            hr = L // n
            x1s = []
            for j in range(n):
                hsh = jnp.concatenate([
                    h_s[pl.ds(r0 + j * hr, hr + 16), i * cw:(i + 1) * cw][8 + sh:8 + sh + hr]
                    for i, sh in enumerate((-1, 1, -2, 2))], axis=1).astype(BF16)
                x1s.append(y_s[pl.ds(r0 + j * hr, hr), :] + _dot(hsh, w2[...]))
            us = None
            if B2_MODE == 1:
                us = [_ln(x1s[j]).astype(BF16) for j in range(n)]
            for j in range(n):
                rows = pl.ds(r0 + j * hr, hr)
                u = us[j] if us is not None else _ln(x1s[j]).astype(BF16)
                u_s[rows, :] = u
                acc = xb_s[rows, :] + x1s[j]
                for f in range(NFA):
                    a = _gelu(_dot(u, w3[:, f * FC:(f + 1) * FC])).astype(BF16)
                    acc = acc + _dot(a, w4[f * FC:(f + 1) * FC, :])
                xc_s[rows, :] = acc
            return c
        with _scope('B2a'):
            jax.lax.fori_loop(0, NSEG, b2a_body, 0)

        def b2b_body(b, c):
            r0 = pl.multiple_of(b * L, L)
            u = u_s[pl.ds(r0, L), :]
            acc = xc_s[pl.ds(r0, L), :]
            for f in range(NFA, F // FC):
                a = _gelu(_dot(u, w3[:, f * FC:(f + 1) * FC])).astype(BF16)
                acc = acc + _dot(a, w4[f * FC:(f + 1) * FC, :])
            xres[pl.ds(r0, L), :] = acc

            @pl.when(rep == 1)
            def _():
                xin[pl.ds(r0, L), :] = acc.astype(BF16)
                pltpu.make_async_copy(xin.at[pl.ds(r0, L), :], out_hbm.at[pl.ds(r0, L), :],
                                      osems.at[b]).start()
            return c
        with _scope('B2b'):
            jax.lax.fori_loop(0, NSEG, b2b_body, 0)
        return carry

    jax.lax.fori_loop(0, 2, rep_body, 0)

    for b in range(NSEG):
        pltpu.make_async_copy(xin.at[pl.ds(b * L, L), :], out_hbm.at[pl.ds(b * L, L), :],
                              osems.at[b]).wait()


@jax.jit
def pallas_interleave_layers__memory_aug_infini_attn__mixer_s_mlp__prompt_kernel(
    A_x, A_wq, A_wk, A_wv, A_wo, A_beta, B_x, B_w1, B_w2, B_w3, B_w4,
):
    x = A_x.reshape(S, D)
    beta = jnp.pad(A_beta.reshape(1, H), ((0, 0), (0, 128 - H)))
    anyspec = pl.BlockSpec(memory_space=pl.ANY)
    scratch = [
        pltpu.VMEM((S, D), BF16),
        pltpu.VMEM((S, D), F32),
        pltpu.VMEM((S, D), F32),
        pltpu.VMEM((S, D), F32),
        pltpu.VMEM((D, D), BF16), pltpu.VMEM((D, D), BF16), pltpu.VMEM((D, D), BF16),
        pltpu.VMEM((D, D), BF16), pltpu.VMEM((D, D), BF16), pltpu.VMEM((D, D), BF16),
        pltpu.VMEM((D, F), BF16), pltpu.VMEM((F, D), BF16),
        pltpu.VMEM((NSEG, NG, L, 128), BF16), pltpu.VMEM((NSEG, NG, L, 128), BF16),
        pltpu.VMEM((NSEG, NG, L, 128), BF16), pltpu.VMEM((NSEG, NG, L, 128), BF16),
        pltpu.VMEM((NSEG, NG, 128, L), BF16),
        pltpu.VMEM((L, D), BF16),
        pltpu.VMEM((2, NG, 128, 128), F32),
        pltpu.VMEM((2, NG, 8, 128), F32),
        pltpu.VMEM((NG, 128, 128), F32),
        pltpu.VMEM((S, D), F32),
        pltpu.VMEM((S + 16, D), F32),
        pltpu.VMEM((S, D), BF16),
        pltpu.SemaphoreType.DMA((NSEG,)),
        pltpu.SemaphoreType.DMA((8,)),
        pltpu.SemaphoreType.DMA((NSEG,)),
    ]
    out = pl.pallas_call(
        _kernel,
        out_shape=jax.ShapeDtypeStruct((S, D), BF16),
        in_specs=[anyspec] * 5 + [pl.BlockSpec(memory_space=pltpu.VMEM)] + [anyspec] * 4,
        out_specs=anyspec,
        scratch_shapes=scratch,
        compiler_params=pltpu.CompilerParams(vmem_limit_bytes=120 * 1024 * 1024),
    )(x, A_wq, A_wk, A_wv, A_wo, beta, B_w1, B_w2, B_w3, B_w4)
    return out.reshape(1, S, D)
```

```python
import math

import jax
import jax.numpy as jnp
import jax.experimental.pallas as pl
import jax.experimental.pallas.tpu as pltpu

S, D, H, F = 2048, 1024, 32, 3584
DH = D // H
NSEG = 4
L = S // NSEG
NG = D // 128
HPG = 128 // DH
EPS = 1e-5
LOG2E = 1.4426950408889634
F32 = jnp.float32
BF16 = jnp.bfloat16
FC = 512
NFA = 2
GU = 8
ORDER = (0, 1, 2, 3)
SPLIT_QKV = 2
SPLIT_OB = 4
SPLIT_B2 = 2
L_LO = 2.0 ** -30
L_HI = 2.0 ** 30


def _lane0(g):
    return g * 128 if isinstance(g, int) else pl.multiple_of(g * 128, 128)


def _ln(x):
    m = jnp.mean(x, axis=-1, keepdims=True)
    xc = x - m
    v = jnp.mean(xc * xc, axis=-1, keepdims=True)
    return xc * jax.lax.rsqrt(v + EPS)


def _gelu(x):
    c = math.sqrt(2.0 / math.pi)
    hx = 0.5 * x
    return hx + hx * jnp.tanh(x * (c + (c * 0.044715) * (x * x)))


def _phi(t):
    return jnp.where(t > 0, t + 1.0, jnp.exp(t))


def _dot(a, b):
    return jnp.dot(a, b, preferred_element_type=F32)


def _dot_nt(a, b):
    return jax.lax.dot_general(a, b, (((1,), (1,)), ((), ())), preferred_element_type=F32)


def _kernel(x_hbm, wq_hbm, wk_hbm, wv_hbm, wo_hbm, beta_ref, w1_hbm, w2_hbm, w3_hbm, w4_hbm,
            out_hbm,
            xin, xres, xb_s, xc_s, wq, wk, wv, wo, w1, w2, w3, w4,
            qs_s, pq_s, k_s, pk_s, vt_s, o_s, m_s, z_s, g_s, y_s, h_s, u_s, xsems, sems, osems):
    xcopies = [pltpu.make_async_copy(x_hbm.at[pl.ds(b * L, L), :], xin.at[pl.ds(b * L, L), :], xsems.at[b])
               for b in range(NSEG)]
    copies = [pltpu.make_async_copy(src, dst, sems.at[i]) for i, (src, dst) in enumerate([
        (wq_hbm, wq), (wk_hbm, wk), (wv_hbm, wv), (wo_hbm, wo),
        (w1_hbm, w1), (w2_hbm, w2), (w3_hbm, w3), (w4_hbm, w4)])]
    xcopies[0].start()
    for c in copies[0:3]:
        c.start()

    gate = jax.nn.sigmoid(beta_ref[...].astype(F32))
    hid = jax.lax.broadcasted_iota(jnp.int32, (128, H), 1)
    rid = jax.lax.broadcasted_iota(jnp.int32, (128, H), 0) // DH
    for g in range(NG):
        col = jnp.sum(jnp.where(hid == g * HPG + rid, gate, 0.0), axis=1, keepdims=True)
        g_s[g] = jnp.broadcast_to(col, (128, 128))

    h_s[pl.ds(0, 8), :] = jnp.zeros((8, D), F32)
    h_s[pl.ds(S + 8, 8), :] = jnp.zeros((8, D), F32)

    scale = DH ** -0.5

    def attention(s, par, truemax, gu, bad0):
        def grp_body(gi, bad):
            bd = (jax.lax.broadcasted_iota(jnp.int32, (128, 128), 1) // DH
                  == jax.lax.broadcasted_iota(jnp.int32, (128, 128), 0) // DH)
            rr = jax.lax.broadcasted_iota(jnp.int32, (128, 128), 0)
            cc = jax.lax.broadcasted_iota(jnp.int32, (128, 128), 1)
            madd = jnp.where(cc < rr, -1e9 * LOG2E, 0.0).astype(F32)
            madd4 = jnp.concatenate([madd] * HPG, axis=1)
            hmask = [jnp.where(jax.lax.broadcasted_iota(jnp.int32, (64, 128), 1) // DH == h,
                               jnp.uint32(0xFFFFFFFF), jnp.uint32(0)) for h in range(HPG)]

            def mem(g):
                pqg = pq_s[s, g]
                pkg = pk_s[s, g]
                mg = m_s[par, g]
                zv = z_s[par, g]
                z16 = jnp.where(jax.lax.broadcasted_iota(jnp.int32, (16, 128), 0)
                                == jax.lax.broadcasted_iota(jnp.int32, (16, 128), 1) // DH, zv[0:1, :], 0.0)
                lhs = jnp.concatenate([mg, z16], axis=0).astype(BF16)
                nd = _dot_nt(lhs, pqg)
                rden = 1.0 / (nd[128:136] + 1e-6)
                if not truemax:
                    upd = _dot(vt_s[s, g], pkg)
                    m_s[1 - par, g] = mg + jnp.where(bd, upd, 0.0)
                    z_s[1 - par, g] = zv + jnp.sum(pkg.astype(F32), axis=0, keepdims=True)
                return nd, rden

            def qk(g, i):
                qiu = pltpu.bitcast(qs_s[s, g, pl.ds(i * 128, 128), :], jnp.uint32)
                qst = jnp.concatenate([pltpu.bitcast(qiu & hmask[h], BF16) for h in range(HPG)], axis=0)
                sd = _dot_nt(k_s[s, g, pl.ds(i * 128, 128), :], qst) + madd4
                if i > 0:
                    so = _dot_nt(k_s[s, g, pl.ds(0, i * 128), :], qst)
                    return jnp.concatenate([so, sd], axis=0)
                return sd

            def sm(st):
                if truemax:
                    p = jnp.exp2(st - jnp.max(st, axis=0, keepdims=True))
                else:
                    p = jnp.exp2(st)
                lsum = jnp.sum(p, axis=0, keepdims=True)
                return [p[:, h * 128:(h + 1) * 128].astype(BF16) for h in range(HPG)], lsum

            def pv(g, i, pbs, rl, nd, rden):
                nk = (i + 1) * 128
                ots = []
                for h in range(HPG):
                    hs = slice(h * 128, (h + 1) * 128)
                    ot = _dot(vt_s[s, g, pl.ds(h * DH, DH), pl.ds(0, nk)], pbs[h])
                    am = nd[h * DH:(h + 1) * DH, i * 128:nk] * rden[h:h + 1, i * 128:nk]
                    gh = g_s[g, pl.ds(h * DH, DH), :]
                    ots.append(gh * am + (1.0 - gh) * (ot * rl[:, hs]))
                res = jnp.concatenate(ots, axis=0)
                o_s[pl.ds(i * 128, 128), pl.ds(_lane0(g), 128)] = res.T.astype(BF16)

            gs = [gi * gu + u for u in range(gu)]
            stages = [(u, i) for u in range(gu) for i in ORDER]
            mems = {}
            sts = {stages[0]: qk(gs[stages[0][0]], stages[0][1])}
            for n, (u, i) in enumerate(stages):
                if u not in mems:
                    mems[u] = mem(gs[u])
                if n + 1 < len(stages):
                    u2, i2 = stages[n + 1]
                    sts[stages[n + 1]] = qk(gs[u2], i2)
                pbs, lsum = sm(sts.pop((u, i)))
                if not truemax:
                    ok = jnp.logical_and(lsum >= L_LO, lsum <= L_HI)
                    bad = jnp.where(ok, bad, 1.0)
                pv(gs[u], i, pbs, 1.0 / lsum, *mems[u])
            return bad
        return jax.lax.fori_loop(0, NG // gu, grp_body, bad0)

    def rep_body(rep, carry):
        def qkv_body(s, c):
            r0 = pl.multiple_of(s * L, L)

            @pl.when(rep == 0)
            def _():
                pltpu.make_async_copy(x_hbm.at[pl.ds(r0, L), :], xin.at[pl.ds(r0, L), :], xsems.at[s]).wait()
                xres[pl.ds(r0, L), :] = xin[pl.ds(r0, L), :].astype(F32)

                @pl.when(s == 0)
                def _():
                    for cp in copies[0:3]:
                        cp.wait()
                    for cp in xcopies[1:] + copies[3:]:
                        cp.start()

            n = SPLIT_QKV
            hr = L // n
            xns = [_ln(xres[pl.ds(r0 + j * hr, hr), :]).astype(BF16) for j in range(n)]
            for j in range(n):
                rows = pl.ds(j * hr, hr)
                xn = xns[j]
                q = _dot(xn, wq[...])
                k = _dot(xn, wk[...])
                v = _dot(xn, wv[...])
                qs = (q * (scale * LOG2E)).astype(BF16)
                pq = _phi(q).astype(BF16)
                kb = k.astype(BF16)
                pk = _phi(k).astype(BF16)
                for g in range(NG):
                    sl = slice(g * 128, (g + 1) * 128)
                    qs_s[s, g, rows, :] = qs[:, sl]
                    pq_s[s, g, rows, :] = pq[:, sl]
                    k_s[s, g, rows, :] = kb[:, sl]
                    pk_s[s, g, rows, :] = pk[:, sl]
                    vt_s[s, g, :, rows] = v[:, sl].T.astype(BF16)
            return c
        jax.lax.fori_loop(0, NSEG, qkv_body, 0)

        m_s[0] = jnp.zeros(m_s.shape[1:], F32)
        z_s[0] = jnp.zeros(z_s.shape[1:], F32)

        def seg_body(s, c):
            r0 = pl.multiple_of(s * L, L)
            par = s % 2
            bad = attention(s, par, False, GU, jnp.zeros((1, HPG * 128), F32))

            @pl.when(jnp.max(bad) > 0.0)
            def _():
                attention(s, par, True, 1, jnp.zeros((1, HPG * 128), F32))

            @pl.when(jnp.logical_and(rep == 0, s == 0))
            def _():
                copies[3].wait()
                copies[4].wait()

            n = SPLIT_OB
            hr = L // n

            def oproj(j):
                ocat = o_s[pl.ds(j * hr, hr), :]
                return xres[pl.ds(r0 + j * hr, hr), :] + _dot(ocat, wo[...])

            def lns(j, xj):
                rows = pl.ds(r0 + j * hr, hr)
                xb_s[rows, :] = xj
                y = _ln(xj)
                y_s[rows, :] = y
                return _ln(y).astype(BF16)

            def w1g(j, yn):
                h_s[pl.ds(r0 + 8 + j * hr, hr), :] = _gelu(_dot(yn, w1[...]))

            xs = [oproj(j) for j in range(n)]
            for j in range(n):
                w1g(j, lns(j, xs[j]))
            return c
        jax.lax.fori_loop(0, NSEG, seg_body, 0)

        @pl.when(rep == 0)
        def _():
            for cp in copies[5:8]:
                cp.wait()

        def b2a_body(b, c):
            r0 = pl.multiple_of(b * L, L)
            cw = D // 4
            n = SPLIT_B2
            hr = L // n
            x1s = []
            for j in range(n):
                hsh = jnp.concatenate([
                    h_s[pl.ds(r0 + j * hr, hr + 16), i * cw:(i + 1) * cw][8 + sh:8 + sh + hr]
                    for i, sh in enumerate((-1, 1, -2, 2))], axis=1).astype(BF16)
                x1s.append(y_s[pl.ds(r0 + j * hr, hr), :] + _dot(hsh, w2[...]))
            for j in range(n):
                rows = pl.ds(r0 + j * hr, hr)
                u = _ln(x1s[j]).astype(BF16)
                u_s[rows, :] = u
                acc = xb_s[rows, :] + x1s[j]
                for f in range(NFA):
                    a = _gelu(_dot(u, w3[:, f * FC:(f + 1) * FC])).astype(BF16)
                    acc = acc + _dot(a, w4[f * FC:(f + 1) * FC, :])
                xc_s[rows, :] = acc
            return c
        jax.lax.fori_loop(0, NSEG, b2a_body, 0)

        def b2b_body(b, c):
            r0 = pl.multiple_of(b * L, L)
            u = u_s[pl.ds(r0, L), :]
            acc = xc_s[pl.ds(r0, L), :]
            for f in range(NFA, F // FC):
                a = _gelu(_dot(u, w3[:, f * FC:(f + 1) * FC])).astype(BF16)
                acc = acc + _dot(a, w4[f * FC:(f + 1) * FC, :])
            xres[pl.ds(r0, L), :] = acc

            @pl.when(rep == 1)
            def _():
                xin[pl.ds(r0, L), :] = acc.astype(BF16)
                pltpu.make_async_copy(xin.at[pl.ds(r0, L), :], out_hbm.at[pl.ds(r0, L), :],
                                      osems.at[b]).start()
            return c
        jax.lax.fori_loop(0, NSEG, b2b_body, 0)
        return carry

    jax.lax.fori_loop(0, 2, rep_body, 0)

    for b in range(NSEG):
        pltpu.make_async_copy(xin.at[pl.ds(b * L, L), :], out_hbm.at[pl.ds(b * L, L), :],
                              osems.at[b]).wait()


@jax.jit
def pallas_interleave_layers__memory_aug_infini_attn__mixer_s_mlp__prompt_kernel(
    A_x, A_wq, A_wk, A_wv, A_wo, A_beta, B_x, B_w1, B_w2, B_w3, B_w4,
):
    x = A_x.reshape(S, D)
    beta = A_beta.reshape(1, H)
    anyspec = pl.BlockSpec(memory_space=pl.ANY)
    scratch = [
        pltpu.VMEM((S, D), BF16),
        pltpu.VMEM((S, D), F32),
        pltpu.VMEM((S, D), F32),
        pltpu.VMEM((S, D), F32),
        pltpu.VMEM((D, D), BF16), pltpu.VMEM((D, D), BF16), pltpu.VMEM((D, D), BF16),
        pltpu.VMEM((D, D), BF16), pltpu.VMEM((D, D), BF16), pltpu.VMEM((D, D), BF16),
        pltpu.VMEM((D, F), BF16), pltpu.VMEM((F, D), BF16),
        pltpu.VMEM((NSEG, NG, L, 128), BF16), pltpu.VMEM((NSEG, NG, L, 128), BF16),
        pltpu.VMEM((NSEG, NG, L, 128), BF16), pltpu.VMEM((NSEG, NG, L, 128), BF16),
        pltpu.VMEM((NSEG, NG, 128, L), BF16),
        pltpu.VMEM((L, D), BF16),
        pltpu.VMEM((2, NG, 128, 128), F32),
        pltpu.VMEM((2, NG, 8, 128), F32),
        pltpu.VMEM((NG, 128, 128), F32),
        pltpu.VMEM((S, D), F32),
        pltpu.VMEM((S + 16, D), F32),
        pltpu.VMEM((S, D), BF16),
        pltpu.SemaphoreType.DMA((NSEG,)),
        pltpu.SemaphoreType.DMA((8,)),
        pltpu.SemaphoreType.DMA((NSEG,)),
    ]
    out = pl.pallas_call(
        _kernel,
        out_shape=jax.ShapeDtypeStruct((S, D), BF16),
        in_specs=[anyspec] * 5 + [pl.BlockSpec(memory_space=pltpu.VMEM)] + [anyspec] * 4,
        out_specs=anyspec,
        scratch_shapes=scratch,
        compiler_params=pltpu.CompilerParams(vmem_limit_bytes=120 * 1024 * 1024),
    )(x, A_wq, A_wk, A_wv, A_wo, beta, B_w1, B_w2, B_w3, B_w4)
    return out.reshape(1, S, D)
```
